```python
import os as _os
_os.environ.setdefault("JAX_PLATFORMS", "cpu")
import jax
import jax.numpy as jnp

def _softmax(x, axis=-1):
    return jax.nn.softmax(x, axis=axis)
def _gelu(x):
    return jax.nn.gelu(x, approximate=True)
def _silu(x):
    return jax.nn.silu(x)
def _sigmoid(x):
    return jax.nn.sigmoid(x)
def _layernorm(x, axis=-1, eps=1e-5):
    m = jnp.mean(x, axis=axis, keepdims=True)
    v = jnp.var(x, axis=axis, keepdims=True)
    return (x - m) / jnp.sqrt(v + eps)
def _scatter_add(tgt, idx, src, axis=0):
    return tgt.at[idx].add(src)
def _segment_sum(src, seg, n):
    return jax.ops.segment_sum(src, seg, n)
class _Rng:
    def __init__(self, key):
        self._k = key
    def _next(self):
        self._k, sub = jax.random.split(self._k)
        return sub
    def normal(self, shape):
        return jax.random.normal(self._next(), shape, dtype=jnp.bfloat16)
    def randint(self, lo, hi, shape):
        return jax.random.randint(self._next(), shape, lo, hi, dtype=jnp.int32)
    def uniform(self, shape, lo=0.0, hi=1.0):
        return jax.random.uniform(self._next(), shape, jnp.bfloat16, lo, hi)
    def permutation(self, n):
        return jax.random.permutation(self._next(), n)


kernel_name = 'concat_heads__spectral_gfnet__mha_block__prompt'

def setup_inputs():
    _rng = _Rng(jax.random.key(int.from_bytes(__import__("os").urandom(4), "little")))
    _w = (lambda a: (lambda t: t.astype(jnp.bfloat16) if jnp.issubdtype(t.dtype, jnp.floating) else t)(jnp.asarray(a)))
    def _A_setup():
        B, S, D = 1, 2048, 576
        Df = D // 2 + 1
        return {
            "x": _w((lambda *s: _rng.normal(s) * 0.05)(B, S, D)),
            "w_r": _w((lambda *s: _rng.normal(s) * 0.05)(S, Df) * 0.02),
            "w_i": _w((lambda *s: _rng.normal(s) * 0.05)(S, Df) * 0.02),
        }
    _A_in = _A_setup()

    def _B_setup():
        B, S, D, H = 1, 2048, 576, 32
        return {
            "x": _w((lambda *s: _rng.normal(s) * 0.1)(B, S, D)),
            "wqkv": _w((lambda *s: _rng.normal(s) * 0.1)(D, 3 * D)),
            "wo": _w((lambda *s: _rng.normal(s) * 0.05)(D, D)),
        }
    _B_in = _B_setup()

    return {
        "A_x": _A_in["x"],
        "A_w_r": _A_in["w_r"],
        "A_w_i": _A_in["w_i"],
        "B_x": _B_in["x"],
        "B_wqkv": _B_in["wqkv"],
        "B_wo": _B_in["wo"],
    }

def reference(A_x, A_w_r, A_w_i, B_x, B_wqkv, B_wo):
    def _A_ref(x, w_r, w_i):
        B, S, D = x.shape
        X = (lambda x, axes=(-2,-1): jnp.fft.rfft2(x.astype(jnp.float32), axes=axes))(x, axes=(-2, -1))
        W = w_r + 1j * w_i
        X = X * W
        y = (lambda x, s, axes=(-2,-1): jnp.fft.irfft2(x, s=s, axes=axes).astype(jnp.bfloat16))(X, (S, D), axes=(-2, -1))
        return y

    def _B_ref(x, wqkv, wo):
        B, S, D = x.shape
        H = 32
        Dh = D // H
        qkv = (lambda x, *d: x.transpose(*d))((x @ wqkv).reshape(B, S, 3, H, Dh), 2, 0, 3, 1, 4)
        q, k, v = qkv[0], qkv[1], qkv[2]
        scores = jnp.einsum("bhqd,bhkd->bhqk", q, k) * (Dh ** -0.5)
        p = _softmax(scores, axis=-1)
        o = jnp.einsum("bhqk,bhkd->bhqd", p, v)
        return (lambda x, *d: x.transpose(*d))(o, 0, 2, 1, 3).reshape(B, S, D) @ wo

    a = _A_ref(A_x, A_w_r, A_w_i)
    b = _B_ref(B_x, B_wqkv, B_wo)
    return jnp.concatenate([a, b], axis=-1)
```

```python
import functools
import math

import numpy as np
import jax
import jax.numpy as jnp
from jax import lax
import jax.experimental.pallas as pl
import jax.experimental.pallas.tpu as pltpu

S = 2048
D = 576
DF = D // 2 + 1
H = 32
DH = 18
HPG = 7
NG = 5
FP = 384
N2 = 16
N1 = S // N2
TQ = 512
KC = 128
NQ = S // TQ
RB = 256
F32 = jnp.float32
BF16 = jnp.bfloat16
TN = (((0,), (0,)), ((), ()))


def _consts():
    d = np.arange(D)[:, None].astype(np.float64)
    kd = np.arange(DF)[None, :].astype(np.float64)
    ang = 2.0 * np.pi * ((d * kd) % D) / D
    fdf = np.zeros((D, 2 * FP), np.float64)
    fdf[:, :DF] = np.cos(ang)
    fdf[:, FP:FP + DF] = -np.sin(ang)
    wgt = np.full((DF,), 2.0)
    wgt[0] = 1.0
    wgt[DF - 1] = 1.0
    scale = 1.0 / (S * D)
    fdi = np.zeros((2 * FP, 640), np.float64)
    fdi[:DF, :D] = (np.cos(ang) * wgt[None, :] * scale).T
    fdi[FP:FP + DF, :D] = (-np.sin(ang) * wgt[None, :] * scale).T
    k1 = np.arange(N1)[:, None]
    n1 = np.arange(N1)[None, :]
    gs = np.zeros((N2, 2 * N1, 2 * N1), np.float64)
    for k2 in range(N2):
        a = 2.0 * np.pi * ((n1 * (N2 * k1 + k2)) % S) / S
        gr = np.cos(a)
        gi = -np.sin(a)
        gs[k2, :N1, :N1] = gr
        gs[k2, :N1, N1:] = -gi
        gs[k2, N1:, :N1] = gi
        gs[k2, N1:, N1:] = gr
    gst = np.transpose(gs, (0, 2, 1))
    cv = lambda a: jnp.asarray(a.astype(np.float32)).astype(BF16)
    return cv(fdf), cv(fdi), cv(gs), cv(gst)


def _cmul_const(xr, xi, c, s):
    eps = 1e-12
    if abs(s) < eps:
        if abs(c - 1.0) < eps:
            return xr, xi
        if abs(c + 1.0) < eps:
            return -xr, -xi
        return xr * c, xi * c
    if abs(c) < eps:
        if abs(s - 1.0) < eps:
            return -xi, xr
        if abs(s + 1.0) < eps:
            return xi, -xr
        return -xi * s, xr * s
    if abs(abs(c) - abs(s)) < eps:
        if c * s > 0:
            return (xr - xi) * c, (xr + xi) * c
        else:
            return (xr + xi) * c, (xi - xr) * c
    return xr * c - xi * s, xr * s + xi * c


def _fft(xs, sign):
    n = len(xs)
    if n == 1:
        return xs
    ev = _fft(xs[0::2], sign)
    od = _fft(xs[1::2], sign)
    out = [None] * n
    for k in range(n // 2):
        ang = sign * 2.0 * math.pi * k / n
        tr, ti = _cmul_const(od[k][0], od[k][1], math.cos(ang), math.sin(ang))
        er, ei = ev[k]
        out[k] = (er + tr, ei + ti)
        out[k + n // 2] = (er - tr, ei - ti)
    return out


def _kernel(xat_hbm, wrt_hbm, wit_hbm, xbt_hbm, wqkv_hbm, wo_hbm, fdf_hbm, fdi_hbm, gs_hbm, gst_hbm,
            out_hbm,
            xat_ref, wrt_ref, wit_ref, xbt_ref, wqkv_ref, wo_ref, fdf_ref, fdi_ref, gs_ref, gst_ref,
            out_scr, in_sems, out_sems,
            k_scr, q_scr, v_scr, o_scr, s_scr, m_scr, x_scr, wr_scr, wi_scr, a_scr, wtmp):
    srcs = [xbt_hbm, wqkv_hbm, xat_hbm, fdf_hbm, wrt_hbm, wit_hbm, gs_hbm, gst_hbm, fdi_hbm, wo_hbm]
    dsts = [xbt_ref, wqkv_ref, xat_ref, fdf_ref, wrt_ref, wit_ref, gs_ref, gst_ref, fdi_ref, wo_ref]
    cps = [pltpu.make_async_copy(s, d, in_sems.at[i]) for i, (s, d) in enumerate(zip(srcs, dsts))]
    for cp in cps:
        cp.start()

    cps[0].wait()
    cps[1].wait()
    qscale = (DH ** -0.5) * math.log2(math.e)
    xbt = xbt_ref[...]
    for g in range(NG):
        wq_g = wqkv_ref[:, 126 * g: 126 * g + 128]
        qt = lax.dot_general(wq_g, xbt, TN, preferred_element_type=F32)
        q_scr[g] = (qt * qscale).astype(BF16)
    vt = lax.dot_general(wqkv_ref[:, 2 * D:3 * D], xbt, TN, preferred_element_type=F32)
    rows32 = lax.broadcasted_iota(jnp.int32, (32, S), 0)
    for h in range(H):
        st = 16 * ((18 * h) // 16)
        off = 18 * h - st
        lrow = 31 if off <= 12 else 0
        win = vt[st:st + 32, :]
        win = jnp.where((rows32 >= off) & (rows32 < off + DH), win,
                        jnp.where(rows32 == lrow, 1.0, 0.0))
        v_scr[h] = win.astype(BF16)
    for g in range(NG):
        wk_g = wqkv_ref[:, D + 126 * g: D + 126 * g + 128]
        k_scr[g] = lax.dot_general(xbt, wk_g, TN, preferred_element_type=F32).astype(BF16)
    o_scr[...] = jnp.zeros_like(o_scr)

    cps[2].wait()
    cps[3].wait()
    cps[4].wait()
    cps[5].wait()
    for w_ref, w_scr in ((wrt_ref, wr_scr), (wit_ref, wi_scr)):
        w_scr[0] = w_ref[0:128, :].astype(F32).T
        w_scr[1] = w_ref[128:256, :].astype(F32).T
        wtmp[...] = jnp.zeros_like(wtmp)
        wtmp[0:DF - 256, :] = w_ref[256:DF, :].astype(F32)
        w_scr[2] = wtmp[...].T
    x_scr[...] = lax.dot_general(xat_ref[...], fdf_ref[...], TN, preferred_element_type=F32)

    def fft_pass(sign):
        def body(r, c):
            r0 = pl.multiple_of(r * 8, 8)
            for ct in range(FP // 128):
                xs = [(x_scr[pl.ds(n2 * N1 + r0, 8), ct * 128:(ct + 1) * 128],
                       x_scr[pl.ds(n2 * N1 + r0, 8), FP + ct * 128:FP + (ct + 1) * 128]) for n2 in range(N2)]
                ys = _fft(xs, sign)
                for k2 in range(N2):
                    x_scr[pl.ds(k2 * N1 + r0, 8), ct * 128:(ct + 1) * 128] = ys[k2][0]
                    x_scr[pl.ds(k2 * N1 + r0, 8), FP + ct * 128:FP + (ct + 1) * 128] = ys[k2][1]
            return c
        lax.fori_loop(0, N1 // 8, body, 0)

    fft_pass(-1)
    cps[6].wait()
    cps[7].wait()
    for k2 in range(N2):
        u = jnp.concatenate([x_scr[k2 * N1:(k2 + 1) * N1, 0:FP], x_scr[k2 * N1:(k2 + 1) * N1, FP:2 * FP]], axis=0)
        t = jnp.dot(gs_ref[k2], u.astype(BF16), preferred_element_type=F32)
        tr, ti = t[:N1], t[N1:]
        wr = jnp.concatenate([wr_scr[c, pl.ds(k2, N1, stride=N2), :] for c in range(3)], axis=1)
        wi = jnp.concatenate([wi_scr[c, pl.ds(k2, N1, stride=N2), :] for c in range(3)], axis=1)
        y = jnp.concatenate([tr * wr - ti * wi, tr * wi + ti * wr], axis=0)
        v = jnp.dot(gst_ref[k2], y.astype(BF16), preferred_element_type=F32)
        x_scr[k2 * N1:(k2 + 1) * N1, 0:FP] = v[:N1]
        x_scr[k2 * N1:(k2 + 1) * N1, FP:2 * FP] = v[N1:]
    fft_pass(+1)
    cps[8].wait()
    a_scr[...] = jnp.dot(x_scr[...].astype(BF16), fdi_ref[...], preferred_element_type=F32)

    N = H * NQ
    nc = S // KC
    rows128 = lax.broadcasted_iota(jnp.int32, (128, TQ), 0)
    rows32q = lax.broadcasted_iota(jnp.int32, (32, TQ), 0)

    def step(i_qk, slot_qk, i_pv, slot_pv):
        h = i_qk // NQ
        qt = i_qk % NQ
        g = h // HPG
        r0 = (h % HPG) * DH
        q0 = pl.multiple_of(qt * TQ, TQ)
        qg = q_scr[g, :, pl.ds(q0, TQ)]
        qm = jnp.where((rows128 >= r0) & (rows128 < r0 + DH), qg, jnp.zeros_like(qg))
        if i_pv is not None:
            hp = i_pv // NQ
            qp0 = pl.multiple_of((i_pv % NQ) * TQ, TQ)
            m = m_scr[slot_pv]
        acc = None
        mx = None
        for c in range(nc):
            s = jnp.dot(k_scr[g, c * KC:(c + 1) * KC, :], qm, preferred_element_type=F32)
            s_scr[slot_qk, c * KC:(c + 1) * KC, :] = s
            sm = jnp.max(s.reshape(KC // 8, 8, TQ), axis=0)
            mx = sm if mx is None else jnp.maximum(mx, sm)
            if i_pv is not None:
                p = jnp.exp2(s_scr[slot_pv, c * KC:(c + 1) * KC, :] - m).astype(BF16)
                o = jnp.dot(v_scr[hp, :, c * KC:(c + 1) * KC], p, preferred_element_type=F32)
                acc = o if acc is None else acc + o
        m_scr[slot_qk] = jnp.max(mx, axis=0, keepdims=True)
        if i_pv is not None:
            off = 2 * (hp % 8)
            st = pl.multiple_of(16 * (hp + hp // 8), 16)
            lrow = jnp.where(off <= 12, 31, 0)
            l = jnp.sum(jnp.where(rows32q == lrow, acc, 0.0), axis=0, keepdims=True)
            on = jnp.where((rows32q >= off) & (rows32q < off + DH), acc / l, 0.0)
            o_scr[pl.ds(st, 32), pl.ds(qp0, TQ)] = o_scr[pl.ds(st, 32), pl.ds(qp0, TQ)] + on

    step(0, 0, None, None)

    def body(j, c):
        i = 2 * j
        step(i + 1, 1, i, 0)
        step(jnp.minimum(i + 2, N - 1), 0, i + 1, 1)
        return c
    lax.fori_loop(0, N // 2, body, 0)

    cps[9].wait()
    wo_sh = jnp.concatenate([jnp.zeros((D, 64), BF16), wo_ref[...]], axis=1)
    ocs = []
    for r in range(S // RB):
        ot = o_scr[:, r * RB:(r + 1) * RB].astype(BF16)
        b = lax.dot_general(ot, wo_sh, TN, preferred_element_type=F32)
        a = a_scr[r * RB:(r + 1) * RB, :]
        out_scr[r * RB:(r + 1) * RB, 0:512] = a[:, 0:512].astype(BF16)
        out_scr[r * RB:(r + 1) * RB, 512:640] = (a[:, 512:640] + b[:, 0:128]).astype(BF16)
        out_scr[r * RB:(r + 1) * RB, 640:1152] = b[:, 128:640].astype(BF16)
        oc = pltpu.make_async_copy(out_scr.at[pl.ds(r * RB, RB)], out_hbm.at[pl.ds(r * RB, RB)], out_sems.at[r])
        oc.start()
        ocs.append(oc)
    for oc in ocs:
        oc.wait()


@jax.jit
def pallas_concat_heads__spectral_gfnet__mha_block__prompt_kernel(A_x, A_w_r, A_w_i, B_x, B_wqkv, B_wo):
    fdf, fdi, gs, gst = _consts()
    args = (A_x.reshape(S, D).T, A_w_r.T, A_w_i.T, B_x.reshape(S, D).T, B_wqkv, B_wo, fdf, fdi, gs, gst)
    out = pl.pallas_call(
        _kernel,
        out_shape=jax.ShapeDtypeStruct((S, 2 * D), BF16),
        in_specs=[pl.BlockSpec(memory_space=pl.ANY)] * len(args),
        out_specs=pl.BlockSpec(memory_space=pl.ANY),
        scratch_shapes=[pltpu.VMEM(a.shape, a.dtype) for a in args] + [
            pltpu.VMEM((S, 2 * D), BF16),
            pltpu.SemaphoreType.DMA((len(args),)),
            pltpu.SemaphoreType.DMA((S // RB,)),
            pltpu.VMEM((NG, S, 128), BF16),
            pltpu.VMEM((NG, 128, S), BF16),
            pltpu.VMEM((H, 32, S), BF16),
            pltpu.VMEM((D, S), F32),
            pltpu.VMEM((2, S, TQ), F32),
            pltpu.VMEM((2, 1, TQ), F32),
            pltpu.VMEM((S, 2 * FP), F32),
            pltpu.VMEM((3, S, 128), F32),
            pltpu.VMEM((3, S, 128), F32),
            pltpu.VMEM((S, 640), F32),
            pltpu.VMEM((128, S), F32),
        ],
        compiler_params=pltpu.CompilerParams(vmem_limit_bytes=110 << 20),
    )(*args)
    return out.reshape(1, S, 2 * D)
```

```python
import functools
import math

import numpy as np
import jax
import jax.numpy as jnp
from jax import lax
import jax.experimental.pallas as pl
import jax.experimental.pallas.tpu as pltpu

S = 2048
D = 576
DF = D // 2 + 1
H = 32
DH = 18
HPG = 7
NG = 5
P = 304
N2 = 16
N1 = S // N2
TQ = 512
KC = 128
NQ = S // TQ
SPI = 8
LAG = 2
RB = 256
CW = 512
NCW = S // CW
F32 = jnp.float32
BF16 = jnp.bfloat16
TN = (((0,), (0,)), ((), ()))
NT = (((1,), (1,)), ((), ()))


def _consts():
    b = np.arange(64)
    th = 2.0 * np.pi / D
    mf = np.zeros((4, 128, 128))
    mi = np.zeros((4, 128, 128))
    sc = 1.0 / (S * D)
    for r in range(1, 5):
        for j in range(32):
            kd = 9 * j + r
            c = np.cos(th * ((b * kd) % D))
            s = np.sin(th * ((b * kd) % D))
            mf[r - 1, j, :64] = c
            mf[r - 1, j, 64:] = s
            mf[r - 1, 64 + j, :64] = -s
            mf[r - 1, 64 + j, 64:] = c
            mi[r - 1, :64, j] = c
            mi[r - 1, :64, 64 + j] = -s
            mi[r - 1, 64:, j] = s
            mi[r - 1, 64:, 64 + j] = c
            kd = 9 * j + 9 - r
            c = np.cos(th * ((b * kd) % D))
            s = np.sin(th * ((b * kd) % D))
            mf[r - 1, 32 + j, :64] = c
            mf[r - 1, 32 + j, 64:] = -s
            mf[r - 1, 96 + j, :64] = -s
            mf[r - 1, 96 + j, 64:] = -c
            mi[r - 1, :64, 32 + j] = c
            mi[r - 1, :64, 96 + j] = -s
            mi[r - 1, 64:, 32 + j] = -s
            mi[r - 1, 64:, 96 + j] = -c
    mi *= 2.0 * sc
    m0f = np.zeros((96, 64))
    m0i = np.zeros((64, 96))
    for j in range(33):
        kd = 9 * j
        c = np.cos(th * ((b * kd) % D))
        s = np.sin(th * ((b * kd) % D))
        m0f[j] = c
        m0f[48 + j] = -s
        w = 1.0 if j in (0, 32) else 2.0
        m0i[:, j] = w * c * sc
        if j not in (0, 32):
            m0i[:, 48 + j] = -w * s * sc
    k1 = np.arange(N1)[:, None]
    n1 = np.arange(N1)[None, :]
    gs = np.zeros((N2, 2 * N1, 2 * N1), np.float64)
    for k2 in range(N2):
        a = 2.0 * np.pi * ((n1 * (N2 * k1 + k2)) % S) / S
        gr = np.cos(a)
        gi = -np.sin(a)
        gs[k2, :N1, :N1] = gr
        gs[k2, :N1, N1:] = -gi
        gs[k2, N1:, :N1] = gi
        gs[k2, N1:, N1:] = gr
    cv = lambda a: jnp.asarray(a.astype(np.float32)).astype(BF16)
    return cv(mf), cv(m0f), cv(mi), cv(m0i), cv(gs)


def _cmul_const(xr, xi, c, s):
    eps = 1e-12
    if abs(s) < eps:
        if abs(c - 1.0) < eps:
            return xr, xi
        if abs(c + 1.0) < eps:
            return -xr, -xi
        return xr * c, xi * c
    if abs(c) < eps:
        if abs(s - 1.0) < eps:
            return -xi, xr
        if abs(s + 1.0) < eps:
            return xi, -xr
        return -xi * s, xr * s
    if abs(abs(c) - abs(s)) < eps:
        if c * s > 0:
            return (xr - xi) * c, (xr + xi) * c
        else:
            return (xr + xi) * c, (xi - xr) * c
    return xr * c - xi * s, xr * s + xi * c


def _fft(xs, sign):
    n = len(xs)
    if n == 1:
        return xs
    ev = _fft(xs[0::2], sign)
    od = _fft(xs[1::2], sign)
    out = [None] * n
    for k in range(n // 2):
        ang = sign * 2.0 * math.pi * k / n
        tr, ti = _cmul_const(od[k][0], od[k][1], math.cos(ang), math.sin(ang))
        er, ei = ev[k]
        out[k] = (er + tr, ei + ti)
        out[k + n // 2] = (er - tr, ei - ti)
    return out


def _sym9(base, e, o):
    c9 = lambda k: math.cos(2.0 * math.pi * k / 9.0)
    s9 = lambda k: math.sin(2.0 * math.pi * k / 9.0)
    h3 = math.sqrt(3.0) / 2.0
    t = base - 0.5 * e[3]
    u = e[1] + e[2] + e[4]
    b3 = base + e[3]
    tot = b3 + u
    cs = {3: b3 - 0.5 * u}
    o3 = o[3] * h3
    sn = {3: (o[1] - o[2] + o[4]) * h3}
    for r in (1, 2, 4):
        cs[r] = t + e[1] * c9(r) + e[2] * c9(2 * r) + e[4] * c9(4 * r)
        acc = o[1] * s9(r) + o[2] * s9(2 * r) + o[4] * s9(4 * r)
        sn[r] = acc + o3 if s9(3 * r) > 0 else acc - o3
    return tot, cs, sn


def _kernel(xat_hbm, wrt_hbm, wit_hbm, xbt_hbm, wqkv_hbm, wo_hbm, mf_hbm, m0f_hbm, mi_hbm, m0i_hbm, gs_hbm,
            out_hbm,
            xat_ref, wrt_ref, wit_ref, xbt_ref, wqkv_ref, wo_ref, mf_ref, m0f_ref, mi_ref, m0i_ref, gs_ref,
            out_scr, in_sems, out_sems,
            k_scr, q_scr, v_scr, o_scr, s_scr, m_scr, xr_scr, xi_scr, wt_scr, w_scr, a_scr, b_scr, wqt_scr, wvt_scr, wk_scr, u_scr, z_scr):
    cp = {}
    order = []

    def add(name, src, dst):
        cp[name] = pltpu.make_async_copy(src, dst, in_sems.at[len(order)])
        order.append(name)

    wcols = [(0, 640), (640, 640), (1280, 448)]
    add("w0", wqkv_hbm.at[:, pl.ds(0, 640)], wqkv_ref.at[:, pl.ds(0, 640)])
    add("xb0", xbt_hbm.at[:, pl.ds(0, CW)], xbt_ref.at[:, pl.ds(0, CW)])
    add("mf", mf_hbm, mf_ref)
    add("m0f", m0f_hbm, m0f_ref)
    add("xa0", xat_hbm.at[:, pl.ds(0, CW)], xat_ref.at[:, pl.ds(0, CW)])
    for c in range(1, NCW):
        add(f"xb{c}", xbt_hbm.at[:, pl.ds(c * CW, CW)], xbt_ref.at[:, pl.ds(c * CW, CW)])
        add(f"xa{c}", xat_hbm.at[:, pl.ds(c * CW, CW)], xat_ref.at[:, pl.ds(c * CW, CW)])
    add("w1", wqkv_hbm.at[:, pl.ds(640, 640)], wqkv_ref.at[:, pl.ds(640, 640)])
    add("w2", wqkv_hbm.at[:, pl.ds(1280, 448)], wqkv_ref.at[:, pl.ds(1280, 448)])
    add("wr", wrt_hbm, wrt_ref)
    add("wi", wit_hbm, wit_ref)
    add("gs", gs_hbm, gs_ref)
    add("mi", mi_hbm, mi_ref)
    add("m0i", m0i_hbm, m0i_ref)
    add("wo", wo_hbm, wo_ref)
    for name in order:
        cp[name].start()

    qscale = (DH ** -0.5) * math.log2(math.e)

    def interleave(mxu_items, vpu_items):
        nm, nv = len(mxu_items), len(vpu_items)
        j = 0
        for i, m in enumerate(mxu_items):
            m()
            tgt = ((i + 1) * nv) // nm
            while j < tgt:
                vpu_items[j]()
                j += 1

    def q_item(c, g):
        def f():
            ls = slice(c * CW, (c + 1) * CW)
            qt = jnp.dot(wqt_scr[g], xbt_ref[:, ls], preferred_element_type=F32)
            q_scr[g, :, ls] = (qt * qscale).astype(BF16)
        return f

    def d9f_item(t, r0):
        def f():
            ts = slice(t * 128, (t + 1) * 128)
            xs = [xat_ref[64 * a + r0:64 * a + r0 + 16, ts].astype(F32) for a in range(9)]
            e = {a: xs[a] + xs[9 - a] for a in range(1, 5)}
            o = {a: xs[9 - a] - xs[a] for a in range(1, 5)}
            a0, cs, sn = _sym9(xs[0], e, o)
            for r in range(1, 5):
                a_scr[128 * (r - 1) + r0:128 * (r - 1) + r0 + 16, ts] = cs[r].astype(BF16)
                a_scr[128 * (r - 1) + 64 + r0:128 * (r - 1) + 64 + r0 + 16, ts] = sn[r].astype(BF16)
            a_scr[512 + r0:512 + r0 + 16, ts] = a0.astype(BF16)
        return f

    def mf_item(c):
        def f():
            ls = slice(c * CW, (c + 1) * CW)
            for r in range(1, 5):
                res = jnp.dot(mf_ref[r - 1], a_scr[128 * (r - 1):128 * r, ls], preferred_element_type=F32)
                xr_scr[64 * (r - 1):64 * r, ls] = res[:64]
                xi_scr[64 * (r - 1):64 * r, ls] = res[64:]
            res = jnp.dot(m0f_ref[...], a_scr[512:576, ls], preferred_element_type=F32)
            xr_scr[256:P, ls] = res[:48]
            xi_scr[256:P, ls] = res[48:]
        return f

    TPC = CW // 128
    cp["w0"].wait()
    for g in range(NG):
        wqt_scr[g] = wqkv_ref[:, 126 * g: 126 * g + 128].T
    for c in range(NCW + 1):
        if c < NCW:
            cp[f"xb{c}"].wait()
        if c == 1:
            cp["mf"].wait()
            cp["m0f"].wait()
        if c >= 1:
            cp[f"xa{c - 1}"].wait()
        mx = [q_item(c, g) for g in range(NG)] if c < NCW else []
        if c >= 2:
            mx.append(mf_item(c - 2))
        vp = [d9f_item(t, r0) for t in range((c - 1) * TPC, c * TPC) for r0 in range(0, 64, 16)] if c >= 1 else []
        if mx:
            interleave(mx, vp)
        else:
            for v in vp:
                v()

    RR = 16

    def _dft4(xs, sign):
        (ar, ai), (br, bi), (cr, ci), (dr, di) = xs
        s0r, s0i = ar + cr, ai + ci
        s1r, s1i = ar - cr, ai - ci
        s2r, s2i = br + dr, bi + di
        s3r, s3i = br - dr, bi - di
        if sign < 0:
            t3r, t3i = s3i, -s3r
        else:
            t3r, t3i = -s3i, s3r
        return [(s0r + s2r, s0i + s2i), (s1r + t3r, s1i + t3i), (s0r - s2r, s0i - s2i), (s1r - t3r, s1i - t3i)]

    def _ld(p0, t):
        return (xr_scr[p0:p0 + RR, t * 128:(t + 1) * 128], xi_scr[p0:p0 + RR, t * 128:(t + 1) * 128])

    def _st(p0, t, v):
        xr_scr[p0:p0 + RR, t * 128:(t + 1) * 128] = v[0]
        xi_scr[p0:p0 + RR, t * 128:(t + 1) * 128] = v[1]

    def _tw(v, k, sign):
        ang = sign * 2.0 * math.pi * k / 16.0
        return _cmul_const(v[0], v[1], math.cos(ang), math.sin(ang))

    def f1_item(p0, b):
        def f():
            ys = _dft4([_ld(p0, 4 * a + b) for a in range(4)], -1)
            for c in range(4):
                _st(p0, 4 * c + b, _tw(ys[c], b * c, -1))
        return f

    def f2_item(p0, c):
        def f():
            ys = _dft4([_ld(p0, 4 * c + b) for b in range(4)], -1)
            for d in range(4):
                u_scr[c + 4 * d, p0:p0 + RR, 0:128] = ys[d][0].astype(BF16)
                u_scr[c + 4 * d, p0:p0 + RR, 128:256] = ys[d][1].astype(BF16)
        return f

    def i1_item(p0, c):
        def f():
            ys = _dft4([_ld(p0, 4 * c + d) for d in range(4)], +1)
            for b in range(4):
                _st(p0, 4 * c + b, _tw(ys[b], b * c, +1))
        return f

    def i2_item(p0, b):
        def f():
            ys = _dft4([_ld(p0, 4 * c + b) for c in range(4)], +1)
            if p0 < 256:
                zr = 128 * (p0 // 64) + p0 % 64
                zi = zr + 64
            else:
                zr = 512 + p0 - 256
                zi = zr + 48
            for a in range(4):
                t = 4 * a + b
                z_scr[zr:zr + RR, t * 128:(t + 1) * 128] = ys[a][0].astype(BF16)
                z_scr[zi:zi + RR, t * 128:(t + 1) * 128] = ys[a][1].astype(BF16)
        return f

    fwd_items = []
    inv_items = []
    for p0 in range(0, P, RR):
        fwd_items += [f1_item(p0, b) for b in range(4)] + [f2_item(p0, c) for c in range(4)]
        inv_items += [i1_item(p0, c) for c in range(4)] + [i2_item(p0, b) for b in range(4)]

    nrc = P // 8

    cp["w1"].wait()
    cp["w2"].wait()
    cp["wr"].wait()
    cp["wi"].wait()
    VW = 256
    wvt_scr[...] = wqkv_ref[:, 2 * D:3 * D].T
    for g in range(NG):
        wk_scr[:, 128 * g:128 * (g + 1)] = wqkv_ref[:, D + 126 * g: D + 126 * g + 128]
    rows32 = lax.broadcasted_iota(jnp.int32, (32, VW), 0)

    def v_item(c):
        def f():
            ls = slice(c * VW, (c + 1) * VW)
            vt = jnp.dot(wvt_scr[...], xbt_ref[:, ls], preferred_element_type=F32)
            for h in range(H):
                st = 16 * ((18 * h) // 16)
                off = 18 * h - st
                lrow = 31 if off <= 12 else 0
                win = vt[st:st + 32, :]
                win = jnp.where((rows32 >= off) & (rows32 < off + DH), win,
                                jnp.where(rows32 == lrow, 1.0, 0.0))
                v_scr[h, :, ls] = win.astype(BF16)
        return f

    def w_item(wi_, t):
        def f():
            w_ref = (wrt_ref, wit_ref)[wi_]
            wt_scr[wi_, t, 0:DF, :] = w_ref[:, t * 128:(t + 1) * 128].astype(F32)
            parts = []
            for r in range(1, 5):
                parts.append(wt_scr[wi_, t, pl.ds(r, 32, stride=9), :])
                parts.append(wt_scr[wi_, t, pl.ds(9 - r, 32, stride=9), :])
            w_scr[wi_, 0, t * 128:(t + 1) * 128, :] = jnp.concatenate(parts[0:4], axis=0).T
            w_scr[wi_, 1, t * 128:(t + 1) * 128, :] = jnp.concatenate(parts[4:8], axis=0).T
            p0 = wt_scr[wi_, t, pl.ds(0, 32, stride=9), :]
            p1 = wt_scr[wi_, t, pl.ds(288 - 7, 8), :]
            rr = lax.broadcasted_iota(jnp.int32, (8, 128), 0)
            p1 = jnp.where(rr == 7, p1, 0.0)
            p1 = pltpu.roll(p1, 1, 0)
            w_scr[wi_, 2, t * 128:(t + 1) * 128, :] = jnp.concatenate(
                [p0, p1, jnp.zeros((88, 128), F32)], axis=0).T
        return f

    def zero_o():
        o_scr[...] = jnp.zeros_like(o_scr)

    w_items = [w_item(wi_, t) for t in range(N2) for wi_ in range(2)]
    f_items = fwd_items
    interleave([mf_item(NCW - 1), v_item(0)], w_items[:8])
    rest = []
    for i in range(len(f_items)):
        rest.append(f_items[i])
        if i % 6 == 0 and 8 + i // 6 < len(w_items):
            rest.append(w_items[8 + i // 6])
    interleave([v_item(c) for c in range(1, S // VW)], rest + [zero_o])

    cp["gs"].wait()

    def g_fwd(k2):
        return lax.dot_general(gs_ref[k2], u_scr[k2], NT, preferred_element_type=F32)

    t_next = g_fwd(0)
    for k2 in range(N2):
        tl = 4 * (k2 % 4) + k2 // 4
        ts = slice(tl * 128, (tl + 1) * 128)
        t = t_next
        if k2 + 1 < N2:
            t_next = g_fwd(k2 + 1)
        tr, ti = t[:N1], t[N1:]
        wr = jnp.concatenate([w_scr[0, c, pl.ds(k2, N1, stride=N2), :] for c in range(3)], axis=1)[:, :P]
        wi = jnp.concatenate([w_scr[1, c, pl.ds(k2, N1, stride=N2), :] for c in range(3)], axis=1)[:, :P]
        y = jnp.concatenate([tr * wr - ti * wi, tr * wi + ti * wr], axis=0).astype(BF16)
        v = lax.dot_general(y, gs_ref[k2], TN, preferred_element_type=F32)
        xr_scr[:, ts] = v[:, :N1]
        xi_scr[:, ts] = v[:, N1:]

    KW = 128

    def k_item(c):
        def f():
            ls = slice(c * KW, (c + 1) * KW)
            kk = lax.dot_general(xbt_ref[:, ls], wk_scr[...], TN, preferred_element_type=F32).astype(BF16)
            for g in range(NG):
                k_scr[g, ls, :] = kk[:, 128 * g:128 * (g + 1)]
        return f

    def mi_item(c):
        def f():
            ls = slice(c * CW, (c + 1) * CW)
            for r in range(1, 5):
                b_scr[128 * (r - 1):128 * r, ls] = jnp.dot(mi_ref[r - 1], z_scr[128 * (r - 1):128 * r, ls],
                                                           preferred_element_type=F32)
            b_scr[512:576, ls] = jnp.dot(m0i_ref[...], z_scr[512:608, ls], preferred_element_type=F32)
        return f

    def d9i_item(t, r0):
        def f():
            ts = slice(t * 128, (t + 1) * 128)
            bre = {r: b_scr[128 * (r - 1) + r0:128 * (r - 1) + r0 + 16, ts] for r in range(1, 5)}
            bim = {r: b_scr[128 * (r - 1) + 64 + r0:128 * (r - 1) + 64 + r0 + 16, ts] for r in range(1, 5)}
            b0 = b_scr[512 + r0:512 + r0 + 16, ts]
            y0, cs, sn = _sym9(b0, bre, bim)
            a_scr[r0:r0 + 16, ts] = y0.astype(BF16)
            for a in range(1, 5):
                a_scr[64 * a + r0:64 * a + r0 + 16, ts] = (cs[a] - sn[a]).astype(BF16)
                a_scr[64 * (9 - a) + r0:64 * (9 - a) + r0 + 16, ts] = (cs[a] + sn[a]).astype(BF16)
        return f

    def tr_item(t):
        def f():
            ts = slice(t * 128, (t + 1) * 128)
            out_scr[ts, 0:D] = a_scr[:, ts].T
        return f

    k_items = [k_item(c) for c in range(S // KW)]
    interleave(k_items[:8], inv_items)
    cp["mi"].wait()
    cp["m0i"].wait()
    for c in range(NCW):
        mi_item(c)()
    cp["wo"].wait()
    tail = []
    for t in range(N2):
        tail += [d9i_item(t, r0) for r0 in range(0, 64, 16)] + [tr_item(t)]
    interleave(k_items[8:], tail)

    N = H * NQ
    nc = S // KC
    rows128 = lax.broadcasted_iota(jnp.int32, (128, TQ), 0)
    rows32q = lax.broadcasted_iota(jnp.int32, (32, TQ), 0)

    def step(i_qk, slot_qk, i_pv, slot_pv):
        h = i_qk // NQ
        qt = i_qk % NQ
        g = h // HPG
        r0 = (h % HPG) * DH
        q0 = pl.multiple_of(qt * TQ, TQ)
        qg = q_scr[g, :, pl.ds(q0, TQ)]
        qm = jnp.where((rows128 >= r0) & (rows128 < r0 + DH), qg, jnp.zeros_like(qg))
        if i_pv is not None:
            hp = i_pv // NQ
            qp0 = pl.multiple_of((i_pv % NQ) * TQ, TQ)
            m = m_scr[slot_pv]
        acc = None
        mx = None
        for c in range(nc + LAG):
            if c < nc:
                s = jnp.dot(k_scr[g, c * KC:(c + 1) * KC, :], qm, preferred_element_type=F32)
                s_scr[slot_qk, c * KC:(c + 1) * KC, :] = s
                sm = jnp.max(s.reshape(KC // 8, 8, TQ), axis=0)
                mx = sm if mx is None else jnp.maximum(mx, sm)
                if c == nc - 1:
                    m_scr[slot_qk] = jnp.max(mx, axis=0, keepdims=True)
            cq = c - LAG
            if i_pv is not None and cq >= 0:
                p = jnp.exp2(s_scr[slot_pv, cq * KC:(cq + 1) * KC, :] - m).astype(BF16)
                o = jnp.dot(v_scr[hp, :, cq * KC:(cq + 1) * KC], p, preferred_element_type=F32)
                acc = o if acc is None else acc + o
        if i_pv is not None:
            off = 2 * (hp % 8)
            st = pl.multiple_of(16 * (hp + hp // 8), 16)
            lrow = jnp.where(off <= 12, 31, 0)
            l = jnp.sum(jnp.where(rows32q == lrow, acc, 0.0), axis=0, keepdims=True)
            on = jnp.where((rows32q >= off) & (rows32q < off + DH), acc / l, 0.0)
            o_scr[pl.ds(st, 32), pl.ds(qp0, TQ)] = o_scr[pl.ds(st, 32), pl.ds(qp0, TQ)] + on

    step(0, 0, None, None)

    def body(j, c):
        i = SPI * j
        for u in range(SPI):
            step(jnp.minimum(i + u + 1, N - 1), (u + 1) % 2, i + u, u % 2)
        return c
    lax.fori_loop(0, N // SPI, body, 0)

    wo_sh = jnp.concatenate([jnp.zeros((D, 64), BF16), wo_ref[...]], axis=1)
    ocs = []
    for r in range(S // RB):
        ot = o_scr[:, r * RB:(r + 1) * RB].astype(BF16)
        b = lax.dot_general(ot, wo_sh, TN, preferred_element_type=F32)
        out_scr[r * RB:(r + 1) * RB, D:2 * D] = b[:, 64:640].astype(BF16)
        oc = pltpu.make_async_copy(out_scr.at[pl.ds(r * RB, RB)], out_hbm.at[pl.ds(r * RB, RB)], out_sems.at[r])
        oc.start()
        ocs.append(oc)
    for oc in ocs:
        oc.wait()


@jax.jit
def pallas_concat_heads__spectral_gfnet__mha_block__prompt_kernel(A_x, A_w_r, A_w_i, B_x, B_wqkv, B_wo):
    consts = _consts()
    args = (A_x.reshape(S, D).T, A_w_r.T, A_w_i.T, B_x.reshape(S, D).T, B_wqkv, B_wo) + consts
    n_in_copies = 3 + 2 * NCW + 8
    out = pl.pallas_call(
        _kernel,
        out_shape=jax.ShapeDtypeStruct((S, 2 * D), BF16),
        in_specs=[pl.BlockSpec(memory_space=pl.ANY)] * len(args),
        out_specs=pl.BlockSpec(memory_space=pl.ANY),
        scratch_shapes=[pltpu.VMEM(a.shape, a.dtype) for a in args] + [
            pltpu.VMEM((S, 2 * D), BF16),
            pltpu.SemaphoreType.DMA((n_in_copies,)),
            pltpu.SemaphoreType.DMA((S // RB,)),
            pltpu.VMEM((NG, S, 128), BF16),
            pltpu.VMEM((NG, 128, S), BF16),
            pltpu.VMEM((H, 32, S), BF16),
            pltpu.VMEM((D, S), F32),
            pltpu.VMEM((2, S, TQ), F32),
            pltpu.VMEM((2, 1, TQ), F32),
            pltpu.VMEM((P, S), F32),
            pltpu.VMEM((P, S), F32),
            pltpu.VMEM((2, N2, 296, 128), F32),
            pltpu.VMEM((2, 3, S, 128), F32),
            pltpu.VMEM((D, S), BF16),
            pltpu.VMEM((D, S), F32),
            pltpu.VMEM((NG, 128, D), BF16),
            pltpu.VMEM((D, D), BF16),
            pltpu.VMEM((D, NG * 128), BF16),
            pltpu.VMEM((N2, P, 256), BF16),
            pltpu.VMEM((608, S), BF16),
        ],
        compiler_params=pltpu.CompilerParams(vmem_limit_bytes=110 << 20),
    )(*args)
    return out.reshape(1, S, 2 * D)
```

```python
import functools
import math

import numpy as np
import jax
import jax.numpy as jnp
from jax import lax
import jax.experimental.pallas as pl
import jax.experimental.pallas.tpu as pltpu

S = 2048
D = 576
DF = D // 2 + 1
H = 32
DH = 18
HPG = 7
NG = 5
P = 304
N2 = 16
N1 = S // N2
TQ = 512
KC = 128
NQ = S // TQ
SPI = 8
LAG = 2
OUT_BLOCKS = (256,) * 7 + (128, 128)
CW = 512
NCW = S // CW
F32 = jnp.float32
BF16 = jnp.bfloat16
TN = (((0,), (0,)), ((), ()))
NT = (((1,), (1,)), ((), ()))


def _consts():
    b = np.arange(64)
    th = 2.0 * np.pi / D
    mf = np.zeros((4, 128, 128))
    mi = np.zeros((4, 128, 128))
    sc = 1.0 / (S * D)
    for r in range(1, 5):
        for j in range(32):
            kd = 9 * j + r
            c = np.cos(th * ((b * kd) % D))
            s = np.sin(th * ((b * kd) % D))
            mf[r - 1, j, :64] = c
            mf[r - 1, j, 64:] = s
            mf[r - 1, 64 + j, :64] = -s
            mf[r - 1, 64 + j, 64:] = c
            mi[r - 1, :64, j] = c
            mi[r - 1, :64, 64 + j] = -s
            mi[r - 1, 64:, j] = s
            mi[r - 1, 64:, 64 + j] = c
            kd = 9 * j + 9 - r
            c = np.cos(th * ((b * kd) % D))
            s = np.sin(th * ((b * kd) % D))
            mf[r - 1, 32 + j, :64] = c
            mf[r - 1, 32 + j, 64:] = -s
            mf[r - 1, 96 + j, :64] = -s
            mf[r - 1, 96 + j, 64:] = -c
            mi[r - 1, :64, 32 + j] = c
            mi[r - 1, :64, 96 + j] = -s
            mi[r - 1, 64:, 32 + j] = -s
            mi[r - 1, 64:, 96 + j] = -c
    mi *= 2.0 * sc
    m0f = np.zeros((96, 64))
    m0i = np.zeros((64, 96))
    for j in range(33):
        kd = 9 * j
        c = np.cos(th * ((b * kd) % D))
        s = np.sin(th * ((b * kd) % D))
        m0f[j] = c
        m0f[48 + j] = -s
        w = 1.0 if j in (0, 32) else 2.0
        m0i[:, j] = w * c * sc
        if j not in (0, 32):
            m0i[:, 48 + j] = -w * s * sc
    k1 = np.arange(N1)[:, None]
    n1 = np.arange(N1)[None, :]
    gs = np.zeros((N2, 2 * N1, 2 * N1), np.float64)
    for k2 in range(N2):
        a = 2.0 * np.pi * ((n1 * (N2 * k1 + k2)) % S) / S
        gr = np.cos(a)
        gi = -np.sin(a)
        gs[k2, :N1, :N1] = gr
        gs[k2, :N1, N1:] = -gi
        gs[k2, N1:, :N1] = gi
        gs[k2, N1:, N1:] = gr
    cv = lambda a: jnp.asarray(a.astype(np.float32)).astype(BF16)
    return cv(mf), cv(m0f), cv(mi), cv(m0i), cv(gs)


def _cmul_const(xr, xi, c, s):
    eps = 1e-12
    if abs(s) < eps:
        if abs(c - 1.0) < eps:
            return xr, xi
        if abs(c + 1.0) < eps:
            return -xr, -xi
        return xr * c, xi * c
    if abs(c) < eps:
        if abs(s - 1.0) < eps:
            return -xi, xr
        if abs(s + 1.0) < eps:
            return xi, -xr
        return -xi * s, xr * s
    if abs(abs(c) - abs(s)) < eps:
        if c * s > 0:
            return (xr - xi) * c, (xr + xi) * c
        else:
            return (xr + xi) * c, (xi - xr) * c
    return xr * c - xi * s, xr * s + xi * c


def _fft(xs, sign):
    n = len(xs)
    if n == 1:
        return xs
    ev = _fft(xs[0::2], sign)
    od = _fft(xs[1::2], sign)
    out = [None] * n
    for k in range(n // 2):
        ang = sign * 2.0 * math.pi * k / n
        tr, ti = _cmul_const(od[k][0], od[k][1], math.cos(ang), math.sin(ang))
        er, ei = ev[k]
        out[k] = (er + tr, ei + ti)
        out[k + n // 2] = (er - tr, ei - ti)
    return out


def _sym9(base, e, o):
    c9 = lambda k: math.cos(2.0 * math.pi * k / 9.0)
    s9 = lambda k: math.sin(2.0 * math.pi * k / 9.0)
    h3 = math.sqrt(3.0) / 2.0
    t = base - 0.5 * e[3]
    u = e[1] + e[2] + e[4]
    b3 = base + e[3]
    tot = b3 + u
    cs = {3: b3 - 0.5 * u}
    o3 = o[3] * h3
    sn = {3: (o[1] - o[2] + o[4]) * h3}
    for r in (1, 2, 4):
        cs[r] = t + e[1] * c9(r) + e[2] * c9(2 * r) + e[4] * c9(4 * r)
        acc = o[1] * s9(r) + o[2] * s9(2 * r) + o[4] * s9(4 * r)
        sn[r] = acc + o3 if s9(3 * r) > 0 else acc - o3
    return tot, cs, sn


def _kernel(one_ref, xat_hbm, wrt_hbm, wit_hbm, xbt_hbm, wqkv_hbm, wo_hbm, mf_hbm, m0f_hbm, mi_hbm, m0i_hbm, gs_hbm,
            out_hbm,
            xat_ref, wrt_ref, wit_ref, xbt_ref, wqkv_ref, wo_ref, mf_ref, m0f_ref, mi_ref, m0i_ref, gs_ref,
            out_scr, in_sems, out_sems,
            k_scr, q_scr, v_scr, o_scr, s_scr, m_scr, xr_scr, xi_scr, wt_scr, w_scr, a_scr, b_scr, wqt_scr, wvt_scr, wk_scr, u_scr, z_scr, xn_scr, wos_scr):
    cp = {}
    order = []

    def add(name, src, dst):
        cp[name] = pltpu.make_async_copy(src, dst, in_sems.at[len(order)])
        order.append(name)

    def lanes(ref, c):
        return ref.at[:, pl.ds(c * CW, CW)]

    add("w0", wqkv_hbm.at[:, pl.ds(0, 640)], wqkv_ref.at[:, pl.ds(0, 640)])
    add("xb0", lanes(xbt_hbm, 0), lanes(xbt_ref, 0))
    add("xa0", lanes(xat_hbm, 0), lanes(xat_ref, 0))
    add("xb1", lanes(xbt_hbm, 1), lanes(xbt_ref, 1))
    add("mf", mf_hbm, mf_ref)
    add("m0f", m0f_hbm, m0f_ref)
    add("xa1", lanes(xat_hbm, 1), lanes(xat_ref, 1))
    add("xb2", lanes(xbt_hbm, 2), lanes(xbt_ref, 2))
    add("w1", wqkv_hbm.at[:, pl.ds(640, 640)], wqkv_ref.at[:, pl.ds(640, 640)])
    add("w2", wqkv_hbm.at[:, pl.ds(1280, 448)], wqkv_ref.at[:, pl.ds(1280, 448)])
    add("xa2", lanes(xat_hbm, 2), lanes(xat_ref, 2))
    add("xb3", lanes(xbt_hbm, 3), lanes(xbt_ref, 3))
    add("xa3", lanes(xat_hbm, 3), lanes(xat_ref, 3))
    add("wr", wrt_hbm, wrt_ref)
    add("wi", wit_hbm, wit_ref)
    add("gs", gs_hbm, gs_ref)
    add("mi", mi_hbm, mi_ref)
    add("m0i", m0i_hbm, m0i_ref)
    add("wo", wo_hbm, wo_ref)
    for name in order:
        cp[name].start()

    qscale = (DH ** -0.5) * math.log2(math.e)
    TPC = CW // 128

    def interleave(mxu_items, vpu_items, frac=0.8):
        nm, nv = len(mxu_items), len(vpu_items)
        span = max(1, int(nm * frac))

        def body(_, carry):
            j = 0
            for i, m in enumerate(mxu_items):
                m()
                tgt = min(nv, ((i + 1) * nv + span - 1) // span)
                while j < tgt:
                    vpu_items[j]()
                    j += 1
            return carry
        lax.fori_loop(0, one_ref[0], body, 0)

    def tl(t):
        return slice(t * 128, (t + 1) * 128)

    def q_item(t, g):
        def f():
            if g < NG - 1:
                qt = jnp.dot(wqt_scr[g], xbt_ref[:, tl(t)], preferred_element_type=F32)
                q_scr[g, :, tl(t)] = (qt * qscale).astype(BF16)
            else:
                qt = jnp.dot(wqt_scr[g, 0:80, :], xbt_ref[:, tl(t)], preferred_element_type=F32)
                q_scr[g, 0:80, tl(t)] = (qt * qscale).astype(BF16)
                q_scr[g, 80:128, tl(t)] = jnp.zeros((48, 128), BF16)
        return f

    def d9f_item(t, r0):
        def f():
            ts = tl(t)
            xs = [xat_ref[64 * a + r0:64 * a + r0 + 16, ts].astype(F32) for a in range(9)]
            e = {a: xs[a] + xs[9 - a] for a in range(1, 5)}
            o = {a: xs[9 - a] - xs[a] for a in range(1, 5)}
            a0, cs, sn = _sym9(xs[0], e, o)
            for r in range(1, 5):
                a_scr[128 * (r - 1) + r0:128 * (r - 1) + r0 + 16, ts] = cs[r].astype(BF16)
                a_scr[128 * (r - 1) + 64 + r0:128 * (r - 1) + 64 + r0 + 16, ts] = sn[r].astype(BF16)
            a_scr[512 + r0:512 + r0 + 16, ts] = a0.astype(BF16)
        return f

    def d9f_items(c):
        return [d9f_item(t, r0) for t in range(c * TPC, (c + 1) * TPC) for r0 in range(0, 64, 16)]

    def mf_item(c, r):
        def f():
            ls = slice(c * CW, (c + 1) * CW)
            if r >= 1:
                res = jnp.dot(mf_ref[r - 1], a_scr[128 * (r - 1):128 * r, ls], preferred_element_type=F32)
                xr_scr[64 * (r - 1):64 * r, ls] = res[:64]
                xi_scr[64 * (r - 1):64 * r, ls] = res[64:]
            else:
                res = jnp.dot(m0f_ref[...], a_scr[512:576, ls], preferred_element_type=F32)
                xr_scr[256:P, ls] = res[:48]
                xi_scr[256:P, ls] = res[48:]
        return f

    def mf_items(c):
        return [mf_item(c, r) for r in range(5)]

    def xn_item(t):
        def f():
            xn_scr[tl(t), :] = xbt_ref[:, tl(t)].T
        return f

    def wv_item(pc):
        def f():
            wvt_scr[144 * pc:144 * (pc + 1), :] = wqkv_ref[:, 2 * D + 144 * pc:2 * D + 144 * (pc + 1)].T
        return f

    def wk_item(g):
        def f():
            wk_scr[:, 128 * g:128 * (g + 1)] = wqkv_ref[:, D + 126 * g: D + 126 * g + 128]
        return f

    RR = 16

    def _dft4(xs, sign):
        (ar, ai), (br, bi), (cr, ci), (dr, di) = xs
        s0r, s0i = ar + cr, ai + ci
        s1r, s1i = ar - cr, ai - ci
        s2r, s2i = br + dr, bi + di
        s3r, s3i = br - dr, bi - di
        if sign < 0:
            t3r, t3i = s3i, -s3r
        else:
            t3r, t3i = -s3i, s3r
        return [(s0r + s2r, s0i + s2i), (s1r + t3r, s1i + t3i), (s0r - s2r, s0i - s2i), (s1r - t3r, s1i - t3i)]

    def _ld(p0, t):
        return (xr_scr[p0:p0 + RR, tl(t)], xi_scr[p0:p0 + RR, tl(t)])

    def _st(p0, t, v):
        xr_scr[p0:p0 + RR, tl(t)] = v[0]
        xi_scr[p0:p0 + RR, tl(t)] = v[1]

    def _tw(v, k, sign):
        ang = sign * 2.0 * math.pi * k / 16.0
        return _cmul_const(v[0], v[1], math.cos(ang), math.sin(ang))

    def f1_item(p0, b):
        def f():
            ys = _dft4([_ld(p0, 4 * a + b) for a in range(4)], -1)
            for c in range(4):
                _st(p0, 4 * c + b, _tw(ys[c], b * c, -1))
        return f

    def f2_item(p0, c):
        def f():
            ys = _dft4([_ld(p0, 4 * c + b) for b in range(4)], -1)
            for d in range(4):
                u_scr[c + 4 * d, p0:p0 + RR, 0:128] = ys[d][0].astype(BF16)
                u_scr[c + 4 * d, p0:p0 + RR, 128:256] = ys[d][1].astype(BF16)
        return f

    def i1_item(p0, c):
        def f():
            ys = _dft4([_ld(p0, 4 * c + d) for d in range(4)], +1)
            for b in range(4):
                _st(p0, 4 * c + b, _tw(ys[b], b * c, +1))
        return f

    def i2_item(p0, b):
        def f():
            ys = _dft4([_ld(p0, 4 * c + b) for c in range(4)], +1)
            if p0 < 256:
                zr = 128 * (p0 // 64) + p0 % 64
                zi = zr + 64
            else:
                zr = 512 + p0 - 256
                zi = zr + 48
            for a in range(4):
                z_scr[zr:zr + RR, tl(4 * a + b)] = ys[a][0].astype(BF16)
                z_scr[zi:zi + RR, tl(4 * a + b)] = ys[a][1].astype(BF16)
        return f

    fwd_items = []
    inv_items = []
    for p0 in range(0, P, RR):
        fwd_items += [f1_item(p0, b) for b in range(4)] + [f2_item(p0, c) for c in range(4)]
        inv_items += [i1_item(p0, c) for c in range(4)] + [i2_item(p0, b) for b in range(4)]

    rows32 = lax.broadcasted_iota(jnp.int32, (32, 128), 0)

    def v_item(t, pc):
        def f():
            vt = jnp.dot(wvt_scr[144 * pc:144 * (pc + 1), :], xbt_ref[:, tl(t)], preferred_element_type=F32)
            for j in range(8):
                off = 2 * j
                lrow = 31 if off <= 12 else 0
                win = vt[16 * j:16 * j + 32, :]
                win = jnp.where((rows32 >= off) & (rows32 < off + DH), win,
                                jnp.where(rows32 == lrow, 1.0, 0.0))
                v_scr[8 * pc + j, :, tl(t)] = win.astype(BF16)
        return f

    def wa_item(wi_, t):
        def f():
            w_ref = (wrt_ref, wit_ref)[wi_]
            wt_scr[wi_, t, 0:DF, :] = w_ref[:, tl(t)].astype(F32)
        return f

    def wb_item(wi_, t, part):
        def f():
            if part < 2:
                parts = []
                for r in (2 * part + 1, 2 * part + 2):
                    parts.append(wt_scr[wi_, t, pl.ds(r, 32, stride=9), :])
                    parts.append(wt_scr[wi_, t, pl.ds(9 - r, 32, stride=9), :])
                w_scr[wi_, part, tl(t), :] = jnp.concatenate(parts, axis=0).T
            else:
                p0 = wt_scr[wi_, t, pl.ds(0, 32, stride=9), :]
                p1 = wt_scr[wi_, t, pl.ds(288 - 7, 8), :]
                rr = lax.broadcasted_iota(jnp.int32, (8, 128), 0)
                p1 = jnp.where(rr == 7, p1, 0.0)
                p1 = pltpu.roll(p1, 1, 0)
                w_scr[wi_, 2, tl(t), :] = jnp.concatenate([p0, p1, jnp.zeros((88, 128), F32)], axis=0).T
        return f

    def zo_item(t):
        def f():
            o_scr[:, tl(t)] = jnp.zeros((D, 128), F32)
        return f

    def k_item(t, g):
        def f():
            k_scr[g, tl(t), :] = jnp.dot(xn_scr[tl(t), :], wk_scr[:, 128 * g:128 * (g + 1)],
                                         preferred_element_type=F32).astype(BF16)
        return f

    def mi_item(c, r):
        def f():
            ls = slice(c * CW, (c + 1) * CW)
            if r >= 1:
                b_scr[128 * (r - 1):128 * r, ls] = jnp.dot(mi_ref[r - 1], z_scr[128 * (r - 1):128 * r, ls],
                                                           preferred_element_type=F32)
            else:
                b_scr[512:576, ls] = jnp.dot(m0i_ref[...], z_scr[512:608, ls], preferred_element_type=F32)
        return f

    def d9i_item(t, r0):
        def f():
            ts = tl(t)
            bre = {r: b_scr[128 * (r - 1) + r0:128 * (r - 1) + r0 + 16, ts] for r in range(1, 5)}
            bim = {r: b_scr[128 * (r - 1) + 64 + r0:128 * (r - 1) + 64 + r0 + 16, ts] for r in range(1, 5)}
            b0 = b_scr[512 + r0:512 + r0 + 16, ts]
            y0, cs, sn = _sym9(b0, bre, bim)
            a_scr[r0:r0 + 16, ts] = y0.astype(BF16)
            for a in range(1, 5):
                a_scr[64 * a + r0:64 * a + r0 + 16, ts] = (cs[a] - sn[a]).astype(BF16)
                a_scr[64 * (9 - a) + r0:64 * (9 - a) + r0 + 16, ts] = (cs[a] + sn[a]).astype(BF16)
        return f

    def tr_item(t):
        def f():
            out_scr[tl(t), 0:D] = a_scr[:, tl(t)].T
        return f

    def q_items(c):
        return [q_item(t, g) for t in range(c * TPC, (c + 1) * TPC) for g in range(NG)]

    def xn_items(c):
        return [xn_item(t) for t in range(c * TPC, (c + 1) * TPC)]

    def merge(la, lb):
        out, j = [], 0
        for i, x in enumerate(la):
            out.append(x)
            tgt = ((i + 1) * len(lb)) // len(la)
            while j < tgt:
                out.append(lb[j])
                j += 1
        return out

    cp["w0"].wait()
    for g in range(NG):
        wqt_scr[g] = wqkv_ref[:, 126 * g: 126 * g + 128].T
    cp["xb0"].wait()
    interleave(q_items(0), xn_items(0))
    cp["xa0"].wait()
    cp["xb1"].wait()
    interleave(q_items(1), d9f_items(0) + xn_items(1))
    cp["mf"].wait()
    cp["m0f"].wait()
    cp["xa1"].wait()
    cp["xb2"].wait()
    interleave(q_items(2) + mf_items(0), d9f_items(1) + xn_items(2))
    cp["w1"].wait()
    cp["w2"].wait()
    cp["xa2"].wait()
    cp["xb3"].wait()
    interleave(q_items(3) + mf_items(1),
               [wv_item(pc) for pc in range(4)] + d9f_items(2) + xn_items(3) + [wk_item(g) for g in range(NG)])

    v_items = [v_item(t, pc) for t in range(N2) for pc in range(4)]
    wa_items = [wa_item(wi_, t) for t in range(N2) for wi_ in range(2)]
    wb_items = [wb_item(wi_, t, part) for t in range(N2) for wi_ in range(2) for part in range(3)]
    cp["xa3"].wait()
    interleave(v_items[:16] + mf_items(2), d9f_items(3))
    cp["wr"].wait()
    cp["wi"].wait()
    interleave(mf_items(3) + v_items[16:26], wa_items, 0.9)
    interleave(v_items[26:], merge(fwd_items, wb_items), 0.9)

    cp["gs"].wait()

    def g_fwd(k2):
        return lax.dot_general(gs_ref[k2], u_scr[k2], NT, preferred_element_type=F32)

    def g_all():
        t_next = g_fwd(0)
        for k2 in range(N2):
            ts = tl(4 * (k2 % 4) + k2 // 4)
            t = t_next
            if k2 + 1 < N2:
                t_next = g_fwd(k2 + 1)
            tr, ti = t[:N1], t[N1:]
            wr = jnp.concatenate([w_scr[0, c, pl.ds(k2, N1, stride=N2), :] for c in range(3)], axis=1)[:, :P]
            wi = jnp.concatenate([w_scr[1, c, pl.ds(k2, N1, stride=N2), :] for c in range(3)], axis=1)[:, :P]
            y = jnp.concatenate([tr * wr - ti * wi, tr * wi + ti * wr], axis=0).astype(BF16)
            v = lax.dot_general(y, gs_ref[k2], TN, preferred_element_type=F32)
            xr_scr[:, ts] = v[:, :N1]
            xi_scr[:, ts] = v[:, N1:]
    interleave([g_all], [])

    k_items = [k_item(t, g) for t in range(N2) for g in range(NG)]
    cp["mi"].wait()
    cp["m0i"].wait()
    cp["wo"].wait()
    interleave(k_items[:32], inv_items, 0.9)
    interleave([mi_item(c, r) for c in range(NCW) for r in range(5)] + k_items[32:36], [])
    interleave(k_items[36:66], [d9i_item(t, r0) for t in range(N2) for r0 in range(0, 64, 16)], 0.9)
    def wos_item():
        wos_scr[...] = jnp.concatenate([jnp.zeros((D, 64), BF16), wo_ref[...]], axis=1)
    interleave(k_items[66:], [tr_item(t) for t in range(N2)] + [wos_item], 0.9)

    N = H * NQ
    nc = S // KC
    rows128 = lax.broadcasted_iota(jnp.int32, (128, TQ), 0)
    rows32q = lax.broadcasted_iota(jnp.int32, (32, TQ), 0)

    def step(i_qk, slot_qk, i_pv, slot_pv):
        h = i_qk // NQ
        qt = i_qk % NQ
        g = h // HPG
        r0 = (h % HPG) * DH
        q0 = pl.multiple_of(qt * TQ, TQ)
        qg = q_scr[g, :, pl.ds(q0, TQ)]
        qm = jnp.where((rows128 >= r0) & (rows128 < r0 + DH), qg, jnp.zeros_like(qg))
        if i_pv is not None:
            hp = i_pv // NQ
            qp0 = pl.multiple_of((i_pv % NQ) * TQ, TQ)
            m = m_scr[slot_pv]
        acc = None
        mx = None
        for c in range(nc + LAG):
            if c < nc:
                s = jnp.dot(k_scr[g, c * KC:(c + 1) * KC, :], qm, preferred_element_type=F32)
                s_scr[slot_qk, c * KC:(c + 1) * KC, :] = s
                sm = jnp.max(s.reshape(KC // 8, 8, TQ), axis=0)
                mx = sm if mx is None else jnp.maximum(mx, sm)
                if c == nc - 1:
                    m_scr[slot_qk] = jnp.max(mx, axis=0, keepdims=True)
            cq = c - LAG
            if i_pv is not None and cq >= 0:
                p = jnp.exp2(s_scr[slot_pv, cq * KC:(cq + 1) * KC, :] - m).astype(BF16)
                o = jnp.dot(v_scr[hp, :, cq * KC:(cq + 1) * KC], p, preferred_element_type=F32)
                acc = o if acc is None else acc + o
        if i_pv is not None:
            off = 2 * (hp % 8)
            st = pl.multiple_of(16 * (hp + hp // 8), 16)
            lrow = jnp.where(off <= 12, 31, 0)
            l = jnp.sum(jnp.where(rows32q == lrow, acc, 0.0), axis=0, keepdims=True)
            pltpu.store(o_scr.at[pl.ds(st, 32), pl.ds(qp0, TQ)], acc / l,
                        mask=(rows32q >= off) & (rows32q < off + DH))

    step(0, 0, None, None)

    def body(j, c):
        i = SPI * j
        for u in range(SPI):
            step(jnp.minimum(i + u + 1, N - 1), (u + 1) % 2, i + u, u % 2)
        return c
    lax.fori_loop(0, N // SPI, body, 0)

    ocs = []
    r0 = 0
    for i, rb in enumerate(OUT_BLOCKS):
        ot = o_scr[:, r0:r0 + rb].astype(BF16)
        b = lax.dot_general(ot, wos_scr[...], TN, preferred_element_type=F32)
        out_scr[r0:r0 + rb, D:2 * D] = b[:, 64:640].astype(BF16)
        oc = pltpu.make_async_copy(out_scr.at[pl.ds(r0, rb)], out_hbm.at[pl.ds(r0, rb)], out_sems.at[i])
        oc.start()
        ocs.append(oc)
        r0 += rb
    for oc in ocs:
        oc.wait()


@jax.jit
def pallas_concat_heads__spectral_gfnet__mha_block__prompt_kernel(A_x, A_w_r, A_w_i, B_x, B_wqkv, B_wo):
    consts = _consts()
    args = (A_x.reshape(S, D).T, A_w_r.T, A_w_i.T, B_x.reshape(S, D).T, B_wqkv, B_wo) + consts
    n_in_copies = 3 + 2 * NCW + 8
    out = pl.pallas_call(
        _kernel,
        out_shape=jax.ShapeDtypeStruct((S, 2 * D), BF16),
        in_specs=[pl.BlockSpec(memory_space=pltpu.SMEM)] + [pl.BlockSpec(memory_space=pl.ANY)] * len(args),
        out_specs=pl.BlockSpec(memory_space=pl.ANY),
        scratch_shapes=[pltpu.VMEM(a.shape, a.dtype) for a in args] + [
            pltpu.VMEM((S, 2 * D), BF16),
            pltpu.SemaphoreType.DMA((n_in_copies,)),
            pltpu.SemaphoreType.DMA((len(OUT_BLOCKS),)),
            pltpu.VMEM((NG, S, 128), BF16),
            pltpu.VMEM((NG, 128, S), BF16),
            pltpu.VMEM((H, 32, S), BF16),
            pltpu.VMEM((D, S), F32),
            pltpu.VMEM((2, S, TQ), F32),
            pltpu.VMEM((2, 1, TQ), F32),
            pltpu.VMEM((P, S), F32),
            pltpu.VMEM((P, S), F32),
            pltpu.VMEM((2, N2, 296, 128), F32),
            pltpu.VMEM((2, 3, S, 128), F32),
            pltpu.VMEM((D, S), BF16),
            pltpu.VMEM((D, S), F32),
            pltpu.VMEM((NG, 128, D), BF16),
            pltpu.VMEM((D, D), BF16),
            pltpu.VMEM((D, NG * 128), BF16),
            pltpu.VMEM((N2, P, 256), BF16),
            pltpu.VMEM((608, S), BF16),
            pltpu.VMEM((S, D), BF16),
            pltpu.VMEM((D, 640), BF16),
        ],
        compiler_params=pltpu.CompilerParams(vmem_limit_bytes=110 << 20),
    )(jnp.ones((1,), jnp.int32), *args)
    return out.reshape(1, S, 2 * D)
```

```python
import math

import numpy as np
import jax
import jax.numpy as jnp
from jax import lax
import jax.experimental.pallas as pl
import jax.experimental.pallas.tpu as pltpu

S = 2048
D = 576
DF = D // 2 + 1
H = 32
DH = 18
HPG = 7
NG = 5
P = 304
N2 = 16
N1 = S // N2
TQ = 512
KC = 128
NQ = S // TQ
SPI = 8
LAG = 2
OUT_BLOCKS = (256,) * 7 + (128, 128)
CW = 512
NCW = S // CW
F32 = jnp.float32
BF16 = jnp.bfloat16
TN = (((0,), (0,)), ((), ()))
NT = (((1,), (1,)), ((), ()))


def _consts():
    b = np.arange(64)
    th = 2.0 * np.pi / D
    mf = np.zeros((4, 128, 128))
    mi = np.zeros((4, 128, 128))
    sc = 1.0 / (S * D)
    for r in range(1, 5):
        for j in range(32):
            kd = 9 * j + r
            c = np.cos(th * ((b * kd) % D))
            s = np.sin(th * ((b * kd) % D))
            mf[r - 1, j, :64] = c
            mf[r - 1, j, 64:] = s
            mf[r - 1, 64 + j, :64] = -s
            mf[r - 1, 64 + j, 64:] = c
            mi[r - 1, :64, j] = c
            mi[r - 1, :64, 64 + j] = -s
            mi[r - 1, 64:, j] = s
            mi[r - 1, 64:, 64 + j] = c
            kd = 9 * j + 9 - r
            c = np.cos(th * ((b * kd) % D))
            s = np.sin(th * ((b * kd) % D))
            mf[r - 1, 32 + j, :64] = c
            mf[r - 1, 32 + j, 64:] = -s
            mf[r - 1, 96 + j, :64] = -s
            mf[r - 1, 96 + j, 64:] = -c
            mi[r - 1, :64, 32 + j] = c
            mi[r - 1, :64, 96 + j] = -s
            mi[r - 1, 64:, 32 + j] = -s
            mi[r - 1, 64:, 96 + j] = -c
    mi *= 2.0 * sc
    m0f = np.zeros((96, 64))
    m0i = np.zeros((64, 96))
    for j in range(33):
        kd = 9 * j
        c = np.cos(th * ((b * kd) % D))
        s = np.sin(th * ((b * kd) % D))
        m0f[j] = c
        m0f[48 + j] = -s
        w = 1.0 if j in (0, 32) else 2.0
        m0i[:, j] = w * c * sc
        if j not in (0, 32):
            m0i[:, 48 + j] = -w * s * sc
    k1 = np.arange(N1)[:, None]
    n1 = np.arange(N1)[None, :]
    gs = np.zeros((N2, 2 * N1, 2 * N1), np.float64)
    for k2 in range(N2):
        a = 2.0 * np.pi * ((n1 * (N2 * k1 + k2)) % S) / S
        gr = np.cos(a)
        gi = -np.sin(a)
        gs[k2, :N1, :N1] = gr
        gs[k2, :N1, N1:] = -gi
        gs[k2, N1:, :N1] = gi
        gs[k2, N1:, N1:] = gr
    cv = lambda a: jnp.asarray(a.astype(np.float32)).astype(BF16)
    return cv(mf), cv(m0f), cv(mi), cv(m0i), cv(gs)


def _cmul_const(xr, xi, c, s):
    eps = 1e-12
    if abs(s) < eps:
        if abs(c - 1.0) < eps:
            return xr, xi
        if abs(c + 1.0) < eps:
            return -xr, -xi
        return xr * c, xi * c
    if abs(c) < eps:
        if abs(s - 1.0) < eps:
            return -xi, xr
        if abs(s + 1.0) < eps:
            return xi, -xr
        return -xi * s, xr * s
    if abs(abs(c) - abs(s)) < eps:
        if c * s > 0:
            return (xr - xi) * c, (xr + xi) * c
        else:
            return (xr + xi) * c, (xi - xr) * c
    return xr * c - xi * s, xr * s + xi * c


def _sym9(base, e, o):
    c9 = lambda k: math.cos(2.0 * math.pi * k / 9.0)
    s9 = lambda k: math.sin(2.0 * math.pi * k / 9.0)
    h3 = math.sqrt(3.0) / 2.0
    t = base - 0.5 * e[3]
    u = e[1] + e[2] + e[4]
    b3 = base + e[3]
    tot = b3 + u
    cs = {3: b3 - 0.5 * u}
    o3 = o[3] * h3
    sn = {3: (o[1] - o[2] + o[4]) * h3}
    for r in (1, 2, 4):
        cs[r] = t + e[1] * c9(r) + e[2] * c9(2 * r) + e[4] * c9(4 * r)
        acc = o[1] * s9(r) + o[2] * s9(2 * r) + o[4] * s9(4 * r)
        sn[r] = acc + o3 if s9(3 * r) > 0 else acc - o3
    return tot, cs, sn


def _kernel(one_ref, xat_hbm, wrt_hbm, wit_hbm, xbt_hbm, wqkv_hbm, wo_hbm, mf_hbm, m0f_hbm, mi_hbm, m0i_hbm, gs_hbm,
            out_hbm,
            xat_ref, wrt_ref, wit_ref, xbt_ref, wqkv_ref, wo_ref, mf_ref, m0f_ref, mi_ref, m0i_ref, gs_ref,
            out_scr, in_sems, out_sems,
            k_scr, q_scr, v_scr, o_scr, s_scr, m_scr, xr_scr, xi_scr, wt_scr, w_scr, a_scr, b_scr, wqt_scr, wvt_scr, wk_scr, u_scr, z_scr, xn_scr, wos_scr):
    cp = {}
    order = []

    def add(name, src, dst):
        cp[name] = pltpu.make_async_copy(src, dst, in_sems.at[len(order)])
        order.append(name)

    def lanes(ref, c):
        return ref.at[:, pl.ds(c * CW, CW)]

    add("w0a", wqkv_hbm.at[:, pl.ds(0, 256)], wqkv_ref.at[:, pl.ds(0, 256)])
    add("xb0", lanes(xbt_hbm, 0), lanes(xbt_ref, 0))
    add("w0b", wqkv_hbm.at[:, pl.ds(256, 384)], wqkv_ref.at[:, pl.ds(256, 384)])
    add("xa0", lanes(xat_hbm, 0), lanes(xat_ref, 0))
    add("xb1", lanes(xbt_hbm, 1), lanes(xbt_ref, 1))
    add("mf", mf_hbm, mf_ref)
    add("m0f", m0f_hbm, m0f_ref)
    add("xa1", lanes(xat_hbm, 1), lanes(xat_ref, 1))
    add("xb2", lanes(xbt_hbm, 2), lanes(xbt_ref, 2))
    add("w1", wqkv_hbm.at[:, pl.ds(640, 640)], wqkv_ref.at[:, pl.ds(640, 640)])
    add("w2", wqkv_hbm.at[:, pl.ds(1280, 448)], wqkv_ref.at[:, pl.ds(1280, 448)])
    add("xa2", lanes(xat_hbm, 2), lanes(xat_ref, 2))
    add("xb3", lanes(xbt_hbm, 3), lanes(xbt_ref, 3))
    add("xa3", lanes(xat_hbm, 3), lanes(xat_ref, 3))
    add("wr", wrt_hbm, wrt_ref)
    add("wi", wit_hbm, wit_ref)
    add("gs", gs_hbm, gs_ref)
    add("mi", mi_hbm, mi_ref)
    add("m0i", m0i_hbm, m0i_ref)
    add("wo", wo_hbm, wo_ref)
    for name in order:
        cp[name].start()

    qscale = (DH ** -0.5) * math.log2(math.e)
    TPC = CW // 128

    def interleave(mxu_items, vpu_items, frac=0.8):
        nm, nv = len(mxu_items), len(vpu_items)
        span = max(1, int(nm * frac))

        def body(_, carry):
            j = 0
            for i, m in enumerate(mxu_items):
                m()
                tgt = min(nv, ((i + 1) * nv + span - 1) // span)
                while j < tgt:
                    vpu_items[j]()
                    j += 1
            return carry
        lax.fori_loop(0, one_ref[0], body, 0)

    def tl(t):
        return slice(t * 128, (t + 1) * 128)

    def q_item(t, g):
        def f():
            if g < NG - 1:
                qt = jnp.dot(wqt_scr[g], xbt_ref[:, tl(t)], preferred_element_type=F32)
                q_scr[g, :, tl(t)] = (qt * qscale).astype(BF16)
            else:
                qt = jnp.dot(wqt_scr[g, 0:80, :], xbt_ref[:, tl(t)], preferred_element_type=F32)
                q_scr[g, 0:80, tl(t)] = (qt * qscale).astype(BF16)
                q_scr[g, 80:128, tl(t)] = jnp.zeros((48, 128), BF16)
        return f

    def d9f_item(t, r0):
        def f():
            ts = tl(t)
            xs = [xat_ref[64 * a + r0:64 * a + r0 + 16, ts].astype(F32) for a in range(9)]
            e = {a: xs[a] + xs[9 - a] for a in range(1, 5)}
            o = {a: xs[9 - a] - xs[a] for a in range(1, 5)}
            a0, cs, sn = _sym9(xs[0], e, o)
            for r in range(1, 5):
                a_scr[128 * (r - 1) + r0:128 * (r - 1) + r0 + 16, ts] = cs[r].astype(BF16)
                a_scr[128 * (r - 1) + 64 + r0:128 * (r - 1) + 64 + r0 + 16, ts] = sn[r].astype(BF16)
            a_scr[512 + r0:512 + r0 + 16, ts] = a0.astype(BF16)
        return f

    def d9f_items(c):
        return [d9f_item(t, r0) for t in range(c * TPC, (c + 1) * TPC) for r0 in range(0, 64, 16)]

    def mf_item(c, r):
        def f():
            ls = slice(c * CW, (c + 1) * CW)
            if r >= 1:
                res = jnp.dot(mf_ref[r - 1], a_scr[128 * (r - 1):128 * r, ls], preferred_element_type=F32)
                xr_scr[64 * (r - 1):64 * r, ls] = res[:64]
                xi_scr[64 * (r - 1):64 * r, ls] = res[64:]
            else:
                res = jnp.dot(m0f_ref[...], a_scr[512:576, ls], preferred_element_type=F32)
                xr_scr[256:P, ls] = res[:48]
                xi_scr[256:P, ls] = res[48:]
        return f

    def mf_items(c):
        return [mf_item(c, r) for r in range(5)]

    def xn_item(t):
        def f():
            xn_scr[tl(t), :] = xbt_ref[:, tl(t)].T
        return f

    def wv_item(pc):
        def f():
            wvt_scr[144 * pc:144 * (pc + 1), :] = wqkv_ref[:, 2 * D + 144 * pc:2 * D + 144 * (pc + 1)].T
        return f

    def wk_item(g):
        def f():
            wk_scr[:, 128 * g:128 * (g + 1)] = wqkv_ref[:, D + 126 * g: D + 126 * g + 128]
        return f

    RR = 16

    def _dft4(xs, sign):
        (ar, ai), (br, bi), (cr, ci), (dr, di) = xs
        s0r, s0i = ar + cr, ai + ci
        s1r, s1i = ar - cr, ai - ci
        s2r, s2i = br + dr, bi + di
        s3r, s3i = br - dr, bi - di
        if sign < 0:
            t3r, t3i = s3i, -s3r
        else:
            t3r, t3i = -s3i, s3r
        return [(s0r + s2r, s0i + s2i), (s1r + t3r, s1i + t3i), (s0r - s2r, s0i - s2i), (s1r - t3r, s1i - t3i)]

    def _ld(p0, t):
        return (xr_scr[p0:p0 + RR, tl(t)], xi_scr[p0:p0 + RR, tl(t)])

    def _st(p0, t, v):
        xr_scr[p0:p0 + RR, tl(t)] = v[0]
        xi_scr[p0:p0 + RR, tl(t)] = v[1]

    def _tw(v, k, sign):
        ang = sign * 2.0 * math.pi * k / 16.0
        return _cmul_const(v[0], v[1], math.cos(ang), math.sin(ang))

    def f1_item(p0, b):
        def f():
            ys = _dft4([_ld(p0, 4 * a + b) for a in range(4)], -1)
            for c in range(4):
                _st(p0, 4 * c + b, _tw(ys[c], b * c, -1))
        return f

    def f2_item(p0, c):
        def f():
            ys = _dft4([_ld(p0, 4 * c + b) for b in range(4)], -1)
            for d in range(4):
                u_scr[c + 4 * d, p0:p0 + RR, 0:128] = ys[d][0].astype(BF16)
                u_scr[c + 4 * d, p0:p0 + RR, 128:256] = ys[d][1].astype(BF16)
        return f

    def i1_item(p0, c):
        def f():
            ys = _dft4([_ld(p0, 4 * c + d) for d in range(4)], +1)
            for b in range(4):
                _st(p0, 4 * c + b, _tw(ys[b], b * c, +1))
        return f

    def i2_item(p0, b):
        def f():
            ys = _dft4([_ld(p0, 4 * c + b) for c in range(4)], +1)
            if p0 < 256:
                zr = 128 * (p0 // 64) + p0 % 64
                zi = zr + 64
            else:
                zr = 512 + p0 - 256
                zi = zr + 48
            for a in range(4):
                z_scr[zr:zr + RR, tl(4 * a + b)] = ys[a][0].astype(BF16)
                z_scr[zi:zi + RR, tl(4 * a + b)] = ys[a][1].astype(BF16)
        return f

    fwd_items = []
    inv_items = []
    for p0 in range(0, P, RR):
        fwd_items += [f1_item(p0, b) for b in range(4)] + [f2_item(p0, c) for c in range(4)]
        inv_items += [i1_item(p0, c) for c in range(4)] + [i2_item(p0, b) for b in range(4)]

    rows32 = lax.broadcasted_iota(jnp.int32, (32, 128), 0)

    def v_item(t, pc):
        def f():
            vt = jnp.dot(wvt_scr[144 * pc:144 * (pc + 1), :], xbt_ref[:, tl(t)], preferred_element_type=F32)
            for j in range(8):
                off = 2 * j
                lrow = 31 if off <= 12 else 0
                win = vt[16 * j:16 * j + 32, :]
                win = jnp.where((rows32 >= off) & (rows32 < off + DH), win,
                                jnp.where(rows32 == lrow, 1.0, 0.0))
                v_scr[8 * pc + j, :, tl(t)] = win.astype(BF16)
        return f

    def wa_item(wi_, t):
        def f():
            w_ref = (wrt_ref, wit_ref)[wi_]
            wt_scr[wi_, t, 0:DF, :] = w_ref[:, tl(t)].astype(F32)
        return f

    def wb_item(wi_, t, part):
        def f():
            if part < 2:
                parts = []
                for r in (2 * part + 1, 2 * part + 2):
                    parts.append(wt_scr[wi_, t, pl.ds(r, 32, stride=9), :])
                    parts.append(wt_scr[wi_, t, pl.ds(9 - r, 32, stride=9), :])
                w_scr[wi_, part, tl(t), :] = jnp.concatenate(parts, axis=0).T
            else:
                p0 = wt_scr[wi_, t, pl.ds(0, 32, stride=9), :]
                p1 = wt_scr[wi_, t, pl.ds(288 - 7, 8), :]
                rr = lax.broadcasted_iota(jnp.int32, (8, 128), 0)
                p1 = jnp.where(rr == 7, p1, 0.0)
                p1 = pltpu.roll(p1, 1, 0)
                w_scr[wi_, 2, tl(t), :] = jnp.concatenate([p0, p1, jnp.zeros((88, 128), F32)], axis=0).T
        return f

    def k_item(t, g):
        def f():
            k_scr[g, tl(t), :] = jnp.dot(xn_scr[tl(t), :], wk_scr[:, 128 * g:128 * (g + 1)],
                                         preferred_element_type=F32).astype(BF16)
        return f

    def mi_item(c, r):
        def f():
            ls = slice(c * CW, (c + 1) * CW)
            if r >= 1:
                b_scr[128 * (r - 1):128 * r, ls] = jnp.dot(mi_ref[r - 1], z_scr[128 * (r - 1):128 * r, ls],
                                                           preferred_element_type=F32)
            else:
                b_scr[512:576, ls] = jnp.dot(m0i_ref[...], z_scr[512:608, ls], preferred_element_type=F32)
        return f

    def d9i_item(t, r0):
        def f():
            ts = tl(t)
            bre = {r: b_scr[128 * (r - 1) + r0:128 * (r - 1) + r0 + 16, ts] for r in range(1, 5)}
            bim = {r: b_scr[128 * (r - 1) + 64 + r0:128 * (r - 1) + 64 + r0 + 16, ts] for r in range(1, 5)}
            b0 = b_scr[512 + r0:512 + r0 + 16, ts]
            y0, cs, sn = _sym9(b0, bre, bim)
            a_scr[r0:r0 + 16, ts] = y0.astype(BF16)
            for a in range(1, 5):
                a_scr[64 * a + r0:64 * a + r0 + 16, ts] = (cs[a] - sn[a]).astype(BF16)
                a_scr[64 * (9 - a) + r0:64 * (9 - a) + r0 + 16, ts] = (cs[a] + sn[a]).astype(BF16)
        return f

    def tr_item(t):
        def f():
            out_scr[tl(t), 0:D] = a_scr[:, tl(t)].T
        return f

    def q_items(c):
        return [q_item(t, g) for t in range(c * TPC, (c + 1) * TPC) for g in range(NG)]

    def xn_items(c):
        return [xn_item(t) for t in range(c * TPC, (c + 1) * TPC)]

    def merge(la, lb):
        out, j = [], 0
        for i, x in enumerate(la):
            out.append(x)
            tgt = ((i + 1) * len(lb)) // len(la)
            while j < tgt:
                out.append(lb[j])
                j += 1
        return out

    def wq_item(g):
        def f():
            wqt_scr[g] = wqkv_ref[:, 126 * g: 126 * g + 128].T
        return f

    cp["w0a"].wait()
    wq_item(0)()
    wq_item(1)()
    cp["xb0"].wait()
    cp["w0b"].wait()
    interleave([q_item(t, g) for g in range(2) for t in range(TPC)], [wq_item(g) for g in range(2, NG)], 0.5)
    interleave([q_item(t, g) for g in range(2, NG) for t in range(TPC)], xn_items(0))
    cp["xa0"].wait()
    cp["xb1"].wait()
    interleave(q_items(1), d9f_items(0) + xn_items(1))
    cp["mf"].wait()
    cp["m0f"].wait()
    cp["xa1"].wait()
    cp["xb2"].wait()
    interleave(q_items(2) + mf_items(0), d9f_items(1) + xn_items(2))
    cp["w1"].wait()
    cp["w2"].wait()
    cp["xa2"].wait()
    cp["xb3"].wait()
    interleave(q_items(3) + mf_items(1),
               [wv_item(pc) for pc in range(4)] + d9f_items(2) + xn_items(3) + [wk_item(g) for g in range(NG)])

    v_items = [v_item(t, pc) for t in range(N2) for pc in range(4)]
    wa_items = [wa_item(wi_, t) for t in range(N2) for wi_ in range(2)]
    wb_items = [wb_item(wi_, t, part) for t in range(N2) for wi_ in range(2) for part in range(3)]
    cp["xa3"].wait()
    interleave(v_items[:16] + mf_items(2), d9f_items(3))
    cp["wr"].wait()
    cp["wi"].wait()
    interleave(mf_items(3) + v_items[16:26], wa_items, 0.9)
    interleave(v_items[26:], merge(fwd_items, wb_items), 0.9)

    cp["gs"].wait()

    def g_fwd(k2):
        return lax.dot_general(gs_ref[k2], u_scr[k2], NT, preferred_element_type=F32)

    def g_all():
        t_next = g_fwd(0)
        for k2 in range(N2):
            ts = tl(4 * (k2 % 4) + k2 // 4)
            t = t_next
            if k2 + 1 < N2:
                t_next = g_fwd(k2 + 1)
            tr, ti = t[:N1], t[N1:]
            wr = jnp.concatenate([w_scr[0, c, pl.ds(k2, N1, stride=N2), :] for c in range(3)], axis=1)[:, :P]
            wi = jnp.concatenate([w_scr[1, c, pl.ds(k2, N1, stride=N2), :] for c in range(3)], axis=1)[:, :P]
            y = jnp.concatenate([tr * wr - ti * wi, tr * wi + ti * wr], axis=0).astype(BF16)
            v = lax.dot_general(y, gs_ref[k2], TN, preferred_element_type=F32)
            xr_scr[:, ts] = v[:, :N1]
            xi_scr[:, ts] = v[:, N1:]
    interleave([g_all], [])

    k_items = [k_item(t, g) for t in range(N2) for g in range(NG)]
    cp["mi"].wait()
    cp["m0i"].wait()
    cp["wo"].wait()
    interleave(k_items[:32], inv_items, 0.9)
    interleave([mi_item(c, r) for c in range(NCW) for r in range(5)] + k_items[32:36], [])
    interleave(k_items[36:66], [d9i_item(t, r0) for t in range(N2) for r0 in range(0, 64, 16)], 0.9)
    def wos_item():
        wos_scr[...] = jnp.concatenate([jnp.zeros((D, 64), BF16), wo_ref[...]], axis=1)
    interleave(k_items[66:], [tr_item(t) for t in range(N2)] + [wos_item], 0.9)

    N = H * NQ
    nc = S // KC
    rows128 = lax.broadcasted_iota(jnp.int32, (128, TQ), 0)
    rows32q = lax.broadcasted_iota(jnp.int32, (32, TQ), 0)

    def step(i_qk, slot_qk, i_pv, slot_pv):
        h = i_qk // NQ
        qt = i_qk % NQ
        g = h // HPG
        r0 = (h % HPG) * DH
        q0 = pl.multiple_of(qt * TQ, TQ)
        qg = q_scr[g, :, pl.ds(q0, TQ)]
        qm = jnp.where((rows128 >= r0) & (rows128 < r0 + DH), qg, jnp.zeros_like(qg))
        if i_pv is not None:
            hp = i_pv // NQ
            qp0 = pl.multiple_of((i_pv % NQ) * TQ, TQ)
            m = m_scr[slot_pv]
        acc = None
        mx = None
        for c in range(nc + LAG):
            if c < nc:
                s = jnp.dot(k_scr[g, c * KC:(c + 1) * KC, :], qm, preferred_element_type=F32)
                s_scr[slot_qk, c * KC:(c + 1) * KC, :] = s
                sm = jnp.max(s.reshape(KC // 8, 8, TQ), axis=0)
                mx = sm if mx is None else jnp.maximum(mx, sm)
                if c == nc - 1:
                    m_scr[slot_qk] = jnp.max(mx, axis=0, keepdims=True)
            cq = c - LAG
            if i_pv is not None and cq >= 0:
                p = jnp.exp2(s_scr[slot_pv, cq * KC:(cq + 1) * KC, :] - m).astype(BF16)
                o = jnp.dot(v_scr[hp, :, cq * KC:(cq + 1) * KC], p, preferred_element_type=F32)
                acc = o if acc is None else acc + o
        if i_pv is not None:
            off = 2 * (hp % 8)
            st = pl.multiple_of(16 * (hp + hp // 8), 16)
            lrow = jnp.where(off <= 12, 31, 0)
            l = jnp.sum(jnp.where(rows32q == lrow, acc, 0.0), axis=0, keepdims=True)
            pltpu.store(o_scr.at[pl.ds(st, 32), pl.ds(qp0, TQ)], acc / l,
                        mask=(rows32q >= off) & (rows32q < off + DH))

    step(0, 0, None, None)

    def body(j, c):
        i = SPI * j
        for u in range(SPI):
            step(jnp.minimum(i + u + 1, N - 1), (u + 1) % 2, i + u, u % 2)
        return c
    lax.fori_loop(0, N // SPI, body, 0)

    ocs = []
    r0 = 0
    for i, rb in enumerate(OUT_BLOCKS):
        ot = o_scr[:, r0:r0 + rb].astype(BF16)
        b = lax.dot_general(ot, wos_scr[...], TN, preferred_element_type=F32)
        out_scr[r0:r0 + rb, D:2 * D] = b[:, 64:640].astype(BF16)
        oc = pltpu.make_async_copy(out_scr.at[pl.ds(r0, rb)], out_hbm.at[pl.ds(r0, rb)], out_sems.at[i])
        oc.start()
        ocs.append(oc)
        r0 += rb
    for oc in ocs:
        oc.wait()


@jax.jit
def pallas_concat_heads__spectral_gfnet__mha_block__prompt_kernel(A_x, A_w_r, A_w_i, B_x, B_wqkv, B_wo):
    consts = _consts()
    args = (A_x.reshape(S, D).T, A_w_r.T, A_w_i.T, B_x.reshape(S, D).T, B_wqkv, B_wo) + consts
    n_in_copies = 4 + 2 * NCW + 8
    out = pl.pallas_call(
        _kernel,
        out_shape=jax.ShapeDtypeStruct((S, 2 * D), BF16),
        in_specs=[pl.BlockSpec(memory_space=pltpu.SMEM)] + [pl.BlockSpec(memory_space=pl.ANY)] * len(args),
        out_specs=pl.BlockSpec(memory_space=pl.ANY),
        scratch_shapes=[pltpu.VMEM(a.shape, a.dtype) for a in args] + [
            pltpu.VMEM((S, 2 * D), BF16),
            pltpu.SemaphoreType.DMA((n_in_copies,)),
            pltpu.SemaphoreType.DMA((len(OUT_BLOCKS),)),
            pltpu.VMEM((NG, S, 128), BF16),
            pltpu.VMEM((NG, 128, S), BF16),
            pltpu.VMEM((H, 32, S), BF16),
            pltpu.VMEM((D, S), F32),
            pltpu.VMEM((2, S, TQ), F32),
            pltpu.VMEM((2, 1, TQ), F32),
            pltpu.VMEM((P, S), F32),
            pltpu.VMEM((P, S), F32),
            pltpu.VMEM((2, N2, 296, 128), F32),
            pltpu.VMEM((2, 3, S, 128), F32),
            pltpu.VMEM((D, S), BF16),
            pltpu.VMEM((D, S), F32),
            pltpu.VMEM((NG, 128, D), BF16),
            pltpu.VMEM((D, D), BF16),
            pltpu.VMEM((D, NG * 128), BF16),
            pltpu.VMEM((N2, P, 256), BF16),
            pltpu.VMEM((608, S), BF16),
            pltpu.VMEM((S, D), BF16),
            pltpu.VMEM((D, 640), BF16),
        ],
        compiler_params=pltpu.CompilerParams(vmem_limit_bytes=110 << 20),
    )(jnp.ones((1,), jnp.int32), *args)
    return out.reshape(1, S, 2 * D)
```
